```python
import os as _os
_os.environ.setdefault("JAX_PLATFORMS", "cpu")
import jax
import jax.numpy as jnp

def _softmax(x, axis=-1):
    return jax.nn.softmax(x, axis=axis)
def _gelu(x):
    return jax.nn.gelu(x, approximate=True)
def _silu(x):
    return jax.nn.silu(x)
def _sigmoid(x):
    return jax.nn.sigmoid(x)
def _layernorm(x, axis=-1, eps=1e-5):
    m = jnp.mean(x, axis=axis, keepdims=True)
    v = jnp.var(x, axis=axis, keepdims=True)
    return (x - m) / jnp.sqrt(v + eps)
def _scatter_add(tgt, idx, src, axis=0):
    return tgt.at[idx].add(src)
def _segment_sum(src, seg, n):
    return jax.ops.segment_sum(src, seg, n)
class _Rng:
    def __init__(self, key):
        self._k = key
    def _next(self):
        self._k, sub = jax.random.split(self._k)
        return sub
    def normal(self, shape):
        return jax.random.normal(self._next(), shape, dtype=jnp.bfloat16)
    def randint(self, lo, hi, shape):
        return jax.random.randint(self._next(), shape, lo, hi, dtype=jnp.int32)
    def uniform(self, shape, lo=0.0, hi=1.0):
        return jax.random.uniform(self._next(), shape, jnp.bfloat16, lo, hi)
    def permutation(self, n):
        return jax.random.permutation(self._next(), n)


kernel_name = 'sequential_preLN__softmax_full_mha__mixer_channel_mlp__prompt'

def setup_inputs():
    _rng = _Rng(jax.random.key(int.from_bytes(__import__("os").urandom(4), "little")))
    _w = (lambda a: (lambda t: t.astype(jnp.bfloat16) if jnp.issubdtype(t.dtype, jnp.floating) else t)(jnp.asarray(a)))
    def _A_setup():
        B, S, D = 1, 2048, 1024
        return {
            "x": _w((lambda *s: _rng.normal(s) * 0.05)(B, S, D)),
            "wqkv": _w((lambda *s: _rng.normal(s) * 0.05)(D, 3 * D)),
            "wo": _w((lambda *s: _rng.normal(s) * 0.05)(D, D)),
        }
    _A_in = _A_setup()

    def _B_setup():
        B, S, D, F = 1, 2048, 1024, 3584
        return {
            "x": _w((lambda *s: _rng.normal(s) * 0.05)(B, S, D)),
            "w1": _w((lambda *s: _rng.normal(s) * 0.8)(D, F) * (D ** -0.5)),
            "b1": _w((lambda *s: _rng.normal(s) * 0.8)(F)),
            "w2": _w((lambda *s: _rng.normal(s) * 0.8)(F, D) * (F ** -0.5)),
            "b2": _w((lambda *s: _rng.normal(s) * 0.05)(D)),
        }
    _B_in = _B_setup()

    return {
        "A_x": _A_in["x"],
        "A_wqkv": _A_in["wqkv"],
        "A_wo": _A_in["wo"],
        "B_x": _B_in["x"],
        "B_w1": _B_in["w1"],
        "B_b1": _B_in["b1"],
        "B_w2": _B_in["w2"],
        "B_b2": _B_in["b2"],
    }

def reference(A_x, A_wqkv, A_wo, B_x, B_w1, B_b1, B_w2, B_b2):
    def _A_ref(x, wqkv, wo):
        B, S, D = x.shape
        H = 32; Dh = D // H
        qkv = (lambda x, *d: x.transpose(*d))((x @ wqkv).reshape(B, S, 3, H, Dh), 2, 0, 3, 1, 4)
        q, k, v = qkv[0], qkv[1], qkv[2]
        scale = Dh ** -0.5
        scores = jnp.einsum("bhqd,bhkd->bhqk", q, k) * scale
        p = _softmax(scores, axis=-1)
        o = jnp.einsum("bhqk,bhkd->bhqd", p, v)
        return (lambda x, *d: x.transpose(*d))(o, 0, 2, 1, 3).reshape(B, S, D) @ wo

    def _B_ref(x, w1, b1, w2, b2):
        y = _layernorm(x, axis=-1)
        h = _gelu(jnp.einsum("bsd,df->bsf", y, w1) + b1)
        return jnp.einsum("bsf,fd->bsd", h, w2) + b2

    x = A_x
    h = x + _A_ref(_layernorm(x, axis=-1), A_wqkv, A_wo)
    h2 = h + _B_ref(_layernorm(h, axis=-1), B_w1, B_b1, B_w2, B_b2)
    return h2
```

```python
import math

import jax
import jax.numpy as jnp
from jax import lax
import jax.experimental.pallas as pl
import jax.experimental.pallas.tpu as pltpu

S = 2048
D = 1024
H = 32
DH = D // H
F = 3584
G = H // 4
TQ = 256
NQ = S // TQ
CK = 128
NC = S // CK
WCH = 512
NWCH = 3 * D // WCH
LAG = 1
GL = 4
EPS = 1e-5
QSCALE = (DH ** -0.5) * math.log2(math.e)

_F32 = jnp.float32
_BF16 = jnp.bfloat16


def _layernorm(x):
    m = jnp.mean(x, axis=-1, keepdims=True)
    xc = x - m
    v = jnp.mean(xc * xc, axis=-1, keepdims=True)
    return xc * lax.rsqrt(v + EPS)


def _kernel(x_hbm, wqkv_hbm, wo_hbm, w1_hbm, b1_ref, w2_hbm, b2_ref, out_hbm,
            x_v, wqkv_v, wo_v, w1_v, w2_v,
            xn_v, k_v, qt_v, vt_v, ot_v,
            s0, s1, s2, s3, m_v,
            h_v, y_v, o_v,
            x_sem, wq_sem, w_sem, o_sem):
    sbuf = (s0, s1, s2, s3)

    def x_copy(i):
        return pltpu.make_async_copy(
            x_hbm.at[pl.ds(i * TQ, TQ), :], x_v.at[pl.ds(i * TQ, TQ), :], x_sem.at[i])

    def wq_copy(c):
        return pltpu.make_async_copy(
            wqkv_hbm.at[:, pl.ds(c * WCH, WCH)], wqkv_v.at[:, pl.ds(c * WCH, WCH)], wq_sem.at[c])

    def w_copies():
        return (pltpu.make_async_copy(wo_hbm, wo_v, w_sem.at[0]),
                pltpu.make_async_copy(w1_hbm, w1_v, w_sem.at[1]),
                pltpu.make_async_copy(w2_hbm, w2_v, w_sem.at[2]))

    def out_copy(i, slot):
        return pltpu.make_async_copy(
            o_v.at[slot], out_hbm.at[pl.ds(i * TQ, TQ), :], o_sem.at[slot])

    x_copy(0).start()
    for c in range(NWCH):
        wq_copy(c).start()
    for i in range(1, NQ):
        x_copy(i).start()

    def ln_x(i):
        row = pl.multiple_of(i * TQ, TQ)
        return _layernorm(x_v[pl.ds(row, TQ), :].astype(_F32)).astype(_BF16)

    def store_qkv_cols(i, r, col0):
        n = r.shape[1]
        row = pl.multiple_of(i * TQ, TQ)
        for sec in range(3):
            lo, hi = max(col0, sec * D), min(col0 + n, (sec + 1) * D)
            if lo >= hi:
                continue
            part = r[:, lo - col0:hi - col0]
            a, b = lo - sec * D, hi - sec * D
            if sec == 0:
                qt_v[i, a:b, :] = (part * QSCALE).T.astype(_BF16)
            elif sec == 1:
                for g in range(a // 128, b // 128):
                    k_v[g, pl.ds(row, TQ), :] = part[:, g * 128 - a:(g + 1) * 128 - a].astype(_BF16)
            else:
                vt_v[i, a:b, :] = part.T.astype(_BF16)

    x_copy(0).wait()
    xn0 = ln_x(0)
    for c in range(NWCH):
        wq_copy(c).wait()
        r = jnp.dot(xn0, wqkv_v[:, c * WCH:(c + 1) * WCH], preferred_element_type=_F32)
        store_qkv_cols(0, r, c * WCH)
    x_copy(1).wait()
    xn_v[1] = ln_x(1)
    for cp in w_copies():
        cp.start()

    def p1_body(i, carry):
        @pl.when(i + 1 < NQ)
        def _():
            x_copy(i + 1).wait()
        r = jnp.dot(xn_v[i % 2], wqkv_v[...], preferred_element_type=_F32)
        store_qkv_cols(i, r, 0)
        xn_v[(i + 1) % 2] = ln_x(jnp.minimum(i + 1, NQ - 1))
        return carry

    lax.fori_loop(1, NQ, p1_body, 0)

    zeros32 = jnp.zeros((DH, TQ), _BF16)

    def q_weights(g, qi, j):
        row = pl.multiple_of((g * 4 + j) * DH, DH)
        qt = qt_v[qi, pl.ds(row, DH), :]
        return jnp.concatenate([qt if jj == j else zeros32 for jj in range(4)], axis=0)

    def qk_chunk(g, w, c, slot, mx):
        s = jnp.dot(k_v[g, c * CK:(c + 1) * CK, :], w, preferred_element_type=_F32)
        sbuf[slot][c * CK:(c + 1) * CK, :] = s
        cm = jnp.max(s.reshape(CK // 8, 8, TQ), axis=0)
        return cm if mx is None else jnp.maximum(mx, cm)

    def sm_chunk(c, slot, m, l):
        p = jnp.exp2(sbuf[slot][c * CK:(c + 1) * CK, :] - m)
        cl = jnp.sum(p.reshape(CK // 8, 8, TQ), axis=0)
        return (cl if l is None else l + cl), p.astype(_BF16)

    def pv_chunk(h, c, pb, o):
        row = pl.multiple_of(h * DH, DH)
        t, off = divmod(c * CK, TQ)
        vt = vt_v[t, pl.ds(row, DH), off:off + CK]
        co = jnp.dot(vt, pb, preferred_element_type=_F32)
        return co if o is None else o + co

    def qk_full(g, qi, j):
        w = q_weights(g, qi, j)
        mx = None
        for c in range(NC):
            mx = qk_chunk(g, w, c, j, mx)
        return jnp.max(mx, axis=0, keepdims=True)

    m_v[0:1, :] = qk_full(0, 0, 0)
    m_v[1:2, :] = qk_full(0, 0, 1)
    NU = G * NQ

    def p2_body(u, carry):
        qi = u // G
        g = u % G
        un = jnp.minimum(u + 1, NU - 1)
        qn = un // G
        gn = un % G
        ms = [m_v[0:1, :], m_v[1:2, :]]
        mx = [None] * 4
        ls = [None] * 4
        os_ = [None] * 4
        ps = {}
        ws = {}
        hist_l = {}
        hist_m = {}
        T = 4 * NC
        for t in range(T + LAG):
            if t < T:
                j, c = divmod(t, NC)
                j2 = (j + 2) % 4
                g2, q2 = (g, qi) if j < 2 else (gn, qn)
                if c == 0:
                    ws[j] = q_weights(g2, q2, j2)
                mx[j] = qk_chunk(g2, ws[j], c, j2, mx[j])
                hist_m[t] = mx[j]
                if c == NC - 1:
                    ms.append(jnp.max(mx[j], axis=0, keepdims=True))
                m = ms[j]
                if t >= GL:
                    m = m + hist_l[t - GL][0:1, :] * 0.0
                    m = m + hist_m[t - GL][0:1, :] * 0.0
                ls[j], ps[t] = sm_chunk(c, j, m, ls[j])
                hist_l[t] = ls[j]
            if t >= LAG:
                j, c = divmod(t - LAG, NC)
                os_[j] = pv_chunk(g * 4 + j, c, ps.pop(t - LAG), os_[j])
                if c == NC - 1:
                    l = jnp.sum(ls[j], axis=0, keepdims=True)
                    row = pl.multiple_of((g * 4 + j) * DH, DH)
                    ot_v[qi, pl.ds(row, DH), :] = (os_[j] * (1.0 / l)).astype(_BF16)
        m_v[0:1, :] = ms[4]
        m_v[1:2, :] = ms[5]
        return carry

    lax.fori_loop(0, NU, p2_body, 0)

    for cp in w_copies():
        cp.wait()

    def proj_ln(i, slot):
        row = pl.multiple_of(i * TQ, TQ)
        o = ot_v[i].T
        a = jnp.dot(o, wo_v[...], preferred_element_type=_F32)
        h = x_v[pl.ds(row, TQ), :].astype(_F32) + a
        h_v[slot] = h
        y_v[slot] = _layernorm(_layernorm(h)).astype(_BF16)

    proj_ln(0, 0)

    def p3_body(i, carry):
        slot = i % 2

        @pl.when(i >= 2)
        def _():
            out_copy(i - 2, slot).wait()

        proj_ln(jnp.minimum(i + 1, NQ - 1), 1 - slot)
        hid = jnp.dot(y_v[slot], w1_v[...], preferred_element_type=_F32)
        hid = jax.nn.gelu(hid + b1_ref[...].astype(_F32), approximate=True).astype(_BF16)
        r = jnp.dot(hid, w2_v[...], preferred_element_type=_F32)
        o_v[slot] = (h_v[slot] + (r + b2_ref[...].astype(_F32))).astype(_BF16)
        out_copy(i, slot).start()
        return carry

    lax.fori_loop(0, NQ, p3_body, 0)
    out_copy(NQ - 2, 0).wait()
    out_copy(NQ - 1, 1).wait()


@jax.jit
def pallas_sequential_preLN__softmax_full_mha__mixer_channel_mlp__prompt_kernel(
    A_x: jax.Array,
    A_wqkv: jax.Array,
    A_wo: jax.Array,
    B_x: jax.Array,
    B_w1: jax.Array,
    B_b1: jax.Array,
    B_w2: jax.Array,
    B_b2: jax.Array,
):
    del B_x
    B = A_x.shape[0]
    assert A_x.shape == (1, S, D) and B == 1
    any_spec = pl.BlockSpec(memory_space=pl.ANY)
    vmem_spec = pl.BlockSpec(memory_space=pltpu.VMEM)
    out = pl.pallas_call(
        _kernel,
        out_shape=jax.ShapeDtypeStruct((S, D), A_x.dtype),
        in_specs=[any_spec, any_spec, any_spec, any_spec, vmem_spec, any_spec, vmem_spec],
        out_specs=any_spec,
        scratch_shapes=[
            pltpu.VMEM((S, D), _BF16),
            pltpu.VMEM((D, 3 * D), _BF16),
            pltpu.VMEM((D, D), _BF16),
            pltpu.VMEM((D, F), _BF16),
            pltpu.VMEM((F, D), _BF16),
            pltpu.VMEM((2, TQ, D), _BF16),
            pltpu.VMEM((G, S, 128), _BF16),
            pltpu.VMEM((NQ, D, TQ), _BF16),
            pltpu.VMEM((NQ, D, TQ), _BF16),
            pltpu.VMEM((NQ, D, TQ), _BF16),
            pltpu.VMEM((S, TQ), _F32),
            pltpu.VMEM((S, TQ), _F32),
            pltpu.VMEM((S, TQ), _F32),
            pltpu.VMEM((S, TQ), _F32),
            pltpu.VMEM((8, TQ), _F32),
            pltpu.VMEM((2, TQ, D), _F32),
            pltpu.VMEM((2, TQ, D), _BF16),
            pltpu.VMEM((2, TQ, D), _BF16),
            pltpu.SemaphoreType.DMA((NQ,)),
            pltpu.SemaphoreType.DMA((NWCH,)),
            pltpu.SemaphoreType.DMA((3,)),
            pltpu.SemaphoreType.DMA((2,)),
        ],
        compiler_params=pltpu.CompilerParams(vmem_limit_bytes=110 * 1024 * 1024),
    )(A_x.reshape(S, D), A_wqkv, A_wo, B_w1, B_b1.reshape(1, F), B_w2, B_b2.reshape(1, D))
    return out.reshape(1, S, D)
```

```python
import math

import jax
import jax.numpy as jnp
from jax import lax
import jax.experimental.pallas as pl
import jax.experimental.pallas.tpu as pltpu

S = 2048
D = 1024
H = 32
DH = D // H
F = 3584
G = H // 4
TQ = 256
NQ = S // TQ
CK = 128
NC = S // CK
WCHUNKS = ((0, 256), (256, 256), (512, 512), (2048, 512), (2560, 512), (1024, 512), (1536, 512))
NWCH = len(WCHUNKS)
LAG = 1
GL = 4
TM = 128
NT = S // TM
GPB = 4
GB = G // GPB
NU = GB * NQ
UB = 4 * GPB
EPS = 1e-5
QSCALE = (DH ** -0.5) * math.log2(math.e)
PEEL3 = True

_F32 = jnp.float32
_BF16 = jnp.bfloat16


def _layernorm(x):
    m = jnp.mean(x, axis=-1, keepdims=True)
    xc = x - m
    v = jnp.mean(xc * xc, axis=-1, keepdims=True)
    return xc * lax.rsqrt(v + EPS)


def _kernel(x_hbm, wqkv_hbm, wo_hbm, w1_hbm, b1_hbm, w2_hbm, b2_hbm, out_hbm,
            x_v, wqkv_v, wo_v, w1_v, w2_v,
            xn_v, k_v, qt_v, vt_v, ot_v,
            s0, s1, s2, s3, m_v,
            h_v, y_v, o_v, b1_v, b2_v,
            in_sem, o_sem):
    sbuf = (s0, s1, s2, s3)

    def x_copy(i):
        return pltpu.make_async_copy(
            x_hbm.at[pl.ds(i * TQ, TQ), :], x_v.at[pl.ds(i * TQ, TQ), :], in_sem.at[i])

    def wq_copy(c):
        c0, n = WCHUNKS[c]
        return pltpu.make_async_copy(
            wqkv_hbm.at[:, pl.ds(c0, n)], wqkv_v.at[:, pl.ds(c0, n)], in_sem.at[NQ + c])

    def w_copies():
        pairs = ((wo_hbm, wo_v), (w1_hbm, w1_v), (w2_hbm, w2_v), (b1_hbm, b1_v), (b2_hbm, b2_v))
        return [pltpu.make_async_copy(src, dst, in_sem.at[NQ + NWCH + k])
                for k, (src, dst) in enumerate(pairs)]

    def out_copy(i, slot):
        return pltpu.make_async_copy(
            o_v.at[slot], out_hbm.at[pl.ds(i * TM, TM), :], o_sem.at[slot])

    x_copy(0).start()
    for c in range(NWCH):
        if c == NWCH - 1:
            x_copy(1).start()
        wq_copy(c).start()
    for i in range(2, NQ):
        x_copy(i).start()
    for cp in w_copies():
        cp.start()

    s2[...] = jnp.zeros_like(s2)
    s3[...] = jnp.zeros_like(s3)
    m_v[...] = jnp.zeros_like(m_v)

    def ln_x(i):
        row = pl.multiple_of(i * TQ, TQ)
        return _layernorm(x_v[pl.ds(row, TQ), :].astype(_F32)).astype(_BF16)

    def store_qkv_cols(i, r, col0):
        n = r.shape[1]
        row = pl.multiple_of(i * TQ, TQ)
        for sec in range(3):
            lo, hi = max(col0, sec * D), min(col0 + n, (sec + 1) * D)
            if lo >= hi:
                continue
            part = r[:, lo - col0:hi - col0]
            a, b = lo - sec * D, hi - sec * D
            if sec == 0:
                qt_v[i, a:b, :] = (part * QSCALE).T.astype(_BF16)
            elif sec == 1:
                for g in range(a // 128, b // 128):
                    k_v[g, pl.ds(row, TQ), :] = part[:, g * 128 - a:(g + 1) * 128 - a].astype(_BF16)
            else:
                vt_v[i, a:b, :] = part.T.astype(_BF16)

    x_copy(0).wait()
    xn0 = ln_x(0)
    for c in range(NWCH):
        wq_copy(c).wait()
        if c == NWCH - 1:
            x_copy(1).wait()
        c0, n = WCHUNKS[c]
        r = jnp.dot(xn0, wqkv_v[:, c0:c0 + n], preferred_element_type=_F32)
        store_qkv_cols(0, r, c0)
    xn_v[1] = ln_x(1)

    def p1_body(i, carry):
        @pl.when(i + 1 < NQ)
        def _():
            x_copy(i + 1).wait()
        xn = xn_v[i % 2]
        for sec in (0, 2, 1):
            r = jnp.dot(xn, wqkv_v[:, sec * D:(sec + 1) * D], preferred_element_type=_F32)
            store_qkv_cols(i, r, sec * D)
        xn_v[(i + 1) % 2] = ln_x(jnp.minimum(i + 1, NQ - 1))
        return carry

    lax.fori_loop(1, NQ, p1_body, 0)

    zeros32 = jnp.zeros((DH, TQ), _BF16)

    def q_weights(h, j, qi):
        row = pl.multiple_of(h * DH, DH)
        qt = qt_v[qi, pl.ds(row, DH), :]
        return jnp.concatenate([qt if jj == j else zeros32 for jj in range(4)], axis=0)

    def qk_chunk(g, w, c, slot, mx):
        s = jnp.dot(k_v[g, c * CK:(c + 1) * CK, :], w, preferred_element_type=_F32)
        sbuf[slot][c * CK:(c + 1) * CK, :] = s
        cm = jnp.max(s.reshape(CK // 8, 8, TQ), axis=0)
        return cm if mx is None else jnp.maximum(mx, cm)

    def sm_chunk(c, slot, m, l):
        p = jnp.exp2(sbuf[slot][c * CK:(c + 1) * CK, :] - m)
        cl = jnp.sum(p.reshape(CK // 8, 8, TQ), axis=0)
        return (cl if l is None else l + cl), p.astype(_BF16)

    def pv_chunk(h, c, pb, o):
        row = pl.multiple_of(h * DH, DH)
        t, off = divmod(c * CK, TQ)
        vt = vt_v[t, pl.ds(row, DH), off:off + CK]
        co = jnp.dot(vt, pb, preferred_element_type=_F32)
        return co if o is None else o + co

    def attn_steps(n_units, cur, prev):
        ms = [m_v[0:1, :], m_v[1:2, :]]
        mx, ls, os_, ps, ws, hist_l, hist_m = {}, {}, {}, {}, {}, {}, {}

        def sm_unit(n):
            return (prev[0] + UB - 2 + n, prev[1]) if n < 2 else (cur[0] + n - 2, cur[1])

        T = n_units * NC
        for t in range(T + LAG):
            if t < T:
                n, c = divmod(t, NC)
                if cur is not None:
                    if c == 0:
                        ws[n] = q_weights(cur[0] + n, n % 4, cur[1])
                    mx[n] = qk_chunk(cur[0] // 4 + n // 4, ws[n], c, n % 4, mx.get(n))
                    hist_m[t] = mx[n]
                    if c == NC - 1:
                        ms.append(jnp.max(mx[n], axis=0, keepdims=True))
                m = ms[n]
                if t >= GL:
                    m = m + hist_l[t - GL][0:1, :] * 0.0
                    if cur is not None:
                        m = m + hist_m[t - GL][0:1, :] * 0.0
                ls[n], ps[t] = sm_chunk(c, (n + 2) % 4, m, ls.get(n))
                hist_l[t] = ls[n]
            if t >= LAG:
                n, c = divmod(t - LAG, NC)
                h, qi = sm_unit(n)
                os_[n] = pv_chunk(h, c, ps.pop(t - LAG), os_.get(n))
                if c == NC - 1:
                    l = jnp.sum(ls[n], axis=0, keepdims=True)
                    row = pl.multiple_of(h * DH, DH)
                    on = (os_[n] * (1.0 / l)).astype(_BF16)
                    for hf in range(TQ // TM):
                        ot_v[qi * (TQ // TM) + hf, pl.ds(row, DH), :] = on[:, hf * TM:(hf + 1) * TM]
        if cur is not None:
            m_v[0:1, :] = ms[n_units]
            m_v[1:2, :] = ms[n_units + 1]

    def p2_body(u, carry):
        up = jnp.maximum(u - 1, 0)
        attn_steps(UB, ((u % GB) * UB, u // GB), ((up % GB) * UB, up // GB))
        return carry

    lax.fori_loop(0, NU, p2_body, 0)

    for cp in w_copies():
        cp.wait()

    def proj_ln(i, slot):
        row = pl.multiple_of(i * TM, TM)
        o = ot_v[i].T
        a = jnp.dot(o, wo_v[...], preferred_element_type=_F32)
        h = x_v[pl.ds(row, TM), :].astype(_F32) + a
        h_v[slot] = h
        y_v[slot] = _layernorm(_layernorm(h)).astype(_BF16)

    proj_ln(0, 0)
    attn_steps(2, None, ((GB - 1) * UB, NQ - 1))

    def p3_step(i, slot, do_proj):
        hid = jnp.dot(y_v[slot], w1_v[...], preferred_element_type=_F32)
        hid = jax.nn.gelu(hid + b1_v[...].astype(_F32).reshape(1, F), approximate=True).astype(_BF16)
        if do_proj:
            proj_ln(jnp.minimum(i + 1, NT - 1), 1 - slot)
        r = jnp.dot(hid, w2_v[...], preferred_element_type=_F32)
        o_v[slot] = (h_v[slot] + (r + b2_v[...].astype(_F32).reshape(1, D))).astype(_BF16)
        out_copy(i, slot).start()

    def p3_body(i, carry):
        slot = i % 2

        @pl.when(i >= 2)
        def _():
            out_copy(i - 2, slot).wait()

        p3_step(i, slot, True)
        return carry

    if PEEL3:
        lax.fori_loop(0, NT - 1, p3_body, 0)
        out_copy(NT - 3, (NT - 1) % 2).wait()
        p3_step(NT - 1, (NT - 1) % 2, False)
    else:
        lax.fori_loop(0, NT, p3_body, 0)
    out_copy(NT - 2, 0).wait()
    out_copy(NT - 1, 1).wait()


@jax.jit
def pallas_sequential_preLN__softmax_full_mha__mixer_channel_mlp__prompt_kernel(
    A_x: jax.Array,
    A_wqkv: jax.Array,
    A_wo: jax.Array,
    B_x: jax.Array,
    B_w1: jax.Array,
    B_b1: jax.Array,
    B_w2: jax.Array,
    B_b2: jax.Array,
):
    del B_x
    assert A_x.shape == (1, S, D)
    any_spec = pl.BlockSpec(memory_space=pl.ANY)
    out = pl.pallas_call(
        _kernel,
        out_shape=jax.ShapeDtypeStruct((S, D), A_x.dtype),
        in_specs=[any_spec] * 7,
        out_specs=any_spec,
        scratch_shapes=[
            pltpu.VMEM((S, D), _BF16),
            pltpu.VMEM((D, 3 * D), _BF16),
            pltpu.VMEM((D, D), _BF16),
            pltpu.VMEM((D, F), _BF16),
            pltpu.VMEM((F, D), _BF16),
            pltpu.VMEM((2, TQ, D), _BF16),
            pltpu.VMEM((G, S, 128), _BF16),
            pltpu.VMEM((NQ, D, TQ), _BF16),
            pltpu.VMEM((NQ, D, TQ), _BF16),
            pltpu.VMEM((NT, D, TM), _BF16),
            pltpu.VMEM((S, TQ), _F32),
            pltpu.VMEM((S, TQ), _F32),
            pltpu.VMEM((S, TQ), _F32),
            pltpu.VMEM((S, TQ), _F32),
            pltpu.VMEM((8, TQ), _F32),
            pltpu.VMEM((2, TM, D), _F32),
            pltpu.VMEM((2, TM, D), _BF16),
            pltpu.VMEM((2, TM, D), _BF16),
            pltpu.VMEM((F,), _BF16),
            pltpu.VMEM((D,), _BF16),
            pltpu.SemaphoreType.DMA((NQ + NWCH + 5,)),
            pltpu.SemaphoreType.DMA((2,)),
        ],
        compiler_params=pltpu.CompilerParams(vmem_limit_bytes=110 * 1024 * 1024),
    )(A_x.reshape(S, D), A_wqkv, A_wo, B_w1, B_b1, B_w2, B_b2)
    return out.reshape(1, S, D)
```

```python
import math

import jax
import jax.numpy as jnp
from jax import lax
import jax.experimental.pallas as pl
import jax.experimental.pallas.tpu as pltpu

S = 2048
D = 1024
H = 32
DH = D // H
F = 3584
G = H // 4
TQ = 256
NQ = S // TQ
CK = 128
NC = S // CK
WCHUNKS = ((0, 256), (256, 256), (512, 512), (2048, 512), (2560, 512), (1024, 512), (1536, 512))
X1POS = 6
NWCH = len(WCHUNKS)
LAG = 1
GL = 4
TM = 128
NT = S // TM
GPB = 4
GB = G // GPB
NU = GB * NQ
UB = 4 * GPB
EPS = 1e-5
QSCALE = (DH ** -0.5) * math.log2(math.e)

_F32 = jnp.float32
_BF16 = jnp.bfloat16


def _layernorm(x):
    m = jnp.mean(x, axis=-1, keepdims=True)
    xc = x - m
    v = jnp.mean(xc * xc, axis=-1, keepdims=True)
    return xc * lax.rsqrt(v + EPS)


def _kernel(x_hbm, wqkv_hbm, wo_hbm, w1_hbm, b1_hbm, w2_hbm, b2_hbm, out_hbm,
            x_v, wqkv_v, wo_v, w1_v, w2_v,
            xn_v, k_v, qt_v, vt_v, ot_v,
            s0, s1, s2, s3, m_v,
            h_v, y_v, o_v, b1_v, b2_v,
            in_sem, o_sem):
    sbuf = (s0, s1, s2, s3)

    def x_copy(i):
        return pltpu.make_async_copy(
            x_hbm.at[pl.ds(i * TQ, TQ), :], x_v.at[pl.ds(i * TQ, TQ), :], in_sem.at[i])

    def wq_copy(c):
        c0, n = WCHUNKS[c]
        return pltpu.make_async_copy(
            wqkv_hbm.at[:, pl.ds(c0, n)], wqkv_v.at[:, pl.ds(c0, n)], in_sem.at[NQ + c])

    def w_copies():
        pairs = ((wo_hbm, wo_v), (w1_hbm, w1_v), (w2_hbm, w2_v), (b1_hbm, b1_v), (b2_hbm, b2_v))
        return [pltpu.make_async_copy(src, dst, in_sem.at[NQ + NWCH + k])
                for k, (src, dst) in enumerate(pairs)]

    def out_copy(i, slot):
        return pltpu.make_async_copy(
            o_v.at[slot], out_hbm.at[pl.ds(i * TM, TM), :], o_sem.at[slot])

    x_copy(0).start()
    for c in range(NWCH):
        if c == X1POS:
            x_copy(1).start()
        wq_copy(c).start()
    for i in range(2, NQ):
        x_copy(i).start()
    for cp in w_copies():
        cp.start()

    s2[...] = jnp.zeros_like(s2)
    s3[...] = jnp.zeros_like(s3)
    m_v[...] = jnp.zeros_like(m_v)

    def ln_x(i):
        row = pl.multiple_of(i * TQ, TQ)
        return _layernorm(x_v[pl.ds(row, TQ), :].astype(_F32)).astype(_BF16)

    def store_qkv_cols(i, r, col0):
        n = r.shape[1]
        row = pl.multiple_of(i * TQ, TQ)
        for sec in range(3):
            lo, hi = max(col0, sec * D), min(col0 + n, (sec + 1) * D)
            if lo >= hi:
                continue
            part = r[:, lo - col0:hi - col0]
            a, b = lo - sec * D, hi - sec * D
            if sec == 0:
                qt_v[i, a:b, :] = (part * QSCALE).T.astype(_BF16)
            elif sec == 1:
                for g in range(a // 128, b // 128):
                    k_v[g, pl.ds(row, TQ), :] = part[:, g * 128 - a:(g + 1) * 128 - a].astype(_BF16)
            else:
                vt_v[i, a:b, :] = part.T.astype(_BF16)

    x_copy(0).wait()
    xn0 = ln_x(0)
    pending = None
    for c in range(NWCH):
        wq_copy(c).wait()
        if c == NWCH - 1:
            x_copy(1).wait()
        c0, n = WCHUNKS[c]
        r = jnp.dot(xn0, wqkv_v[:, c0:c0 + n], preferred_element_type=_F32)
        if pending is not None:
            store_qkv_cols(0, *pending)
            pending = None
        if c < NWCH - 1 and not (D <= c0 < 2 * D):
            pending = (r, c0)
        else:
            store_qkv_cols(0, r, c0)
    xn_v[1] = ln_x(1)

    def p1_body(i, carry):
        @pl.when(i + 1 < NQ)
        def _():
            x_copy(i + 1).wait()
        xn = xn_v[i % 2]
        for sec in (0, 2, 1):
            r = jnp.dot(xn, wqkv_v[:, sec * D:(sec + 1) * D], preferred_element_type=_F32)
            store_qkv_cols(i, r, sec * D)
        xn_v[(i + 1) % 2] = ln_x(jnp.minimum(i + 1, NQ - 1))
        return carry

    lax.fori_loop(1, NQ, p1_body, 0)

    zeros32 = jnp.zeros((DH, TQ), _BF16)

    def q_weights(h, j, qi):
        row = pl.multiple_of(h * DH, DH)
        qt = qt_v[qi, pl.ds(row, DH), :]
        return jnp.concatenate([qt if jj == j else zeros32 for jj in range(4)], axis=0)

    def qk_chunk(g, w, c, slot, mx):
        s = jnp.dot(k_v[g, c * CK:(c + 1) * CK, :], w, preferred_element_type=_F32)
        sbuf[slot][c * CK:(c + 1) * CK, :] = s
        cm = jnp.max(s.reshape(CK // 8, 8, TQ), axis=0)
        return cm if mx is None else jnp.maximum(mx, cm)

    def sm_chunk(c, slot, m, l):
        p = jnp.exp2(sbuf[slot][c * CK:(c + 1) * CK, :] - m)
        cl = jnp.sum(p.reshape(CK // 8, 8, TQ), axis=0)
        return (cl if l is None else l + cl), p.astype(_BF16)

    def pv_chunk(h, c, pb, o):
        row = pl.multiple_of(h * DH, DH)
        t, off = divmod(c * CK, TQ)
        vt = vt_v[t, pl.ds(row, DH), off:off + CK]
        co = jnp.dot(vt, pb, preferred_element_type=_F32)
        return co if o is None else o + co

    def attn_steps(n_units, cur, prev):
        ms = [m_v[0:1, :], m_v[1:2, :]]
        mx, ls, os_, ps, ws, hist_l, hist_m = {}, {}, {}, {}, {}, {}, {}

        def sm_unit(n):
            return (prev[0] + UB - 2 + n, prev[1]) if n < 2 else (cur[0] + n - 2, cur[1])

        T = n_units * NC
        for t in range(T + LAG):
            if t < T:
                n, c = divmod(t, NC)
                if cur is not None:
                    if c == 0:
                        ws[n] = q_weights(cur[0] + n, n % 4, cur[1])
                    mx[n] = qk_chunk(cur[0] // 4 + n // 4, ws[n], c, n % 4, mx.get(n))
                    hist_m[t] = mx[n]
                    if c == NC - 1:
                        ms.append(jnp.max(mx[n], axis=0, keepdims=True))
                m = ms[n]
                if t >= GL:
                    m = m + hist_l[t - GL][0:1, :] * 0.0
                    if cur is not None:
                        m = m + hist_m[t - GL][0:1, :] * 0.0
                ls[n], ps[t] = sm_chunk(c, (n + 2) % 4, m, ls.get(n))
                hist_l[t] = ls[n]
            if t >= LAG:
                n, c = divmod(t - LAG, NC)
                h, qi = sm_unit(n)
                os_[n] = pv_chunk(h, c, ps.pop(t - LAG), os_.get(n))
                if c == NC - 1:
                    l = jnp.sum(ls[n], axis=0, keepdims=True)
                    row = pl.multiple_of(h * DH, DH)
                    on = (os_[n] * (1.0 / l)).astype(_BF16)
                    for hf in range(TQ // TM):
                        ot_v[qi * (TQ // TM) + hf, pl.ds(row, DH), :] = on[:, hf * TM:(hf + 1) * TM]
        if cur is not None:
            m_v[0:1, :] = ms[n_units]
            m_v[1:2, :] = ms[n_units + 1]

    def p2_body(u, carry):
        up = jnp.maximum(u - 1, 0)
        attn_steps(UB, ((u % GB) * UB, u // GB), ((up % GB) * UB, up // GB))
        return carry

    lax.fori_loop(0, NU, p2_body, 0)

    for cp in w_copies():
        cp.wait()

    def proj_ln(i, slot):
        row = pl.multiple_of(i * TM, TM)
        o = ot_v[i].T
        a = jnp.dot(o, wo_v[...], preferred_element_type=_F32)
        h = x_v[pl.ds(row, TM), :].astype(_F32) + a
        h_v[slot] = h
        y_v[slot] = _layernorm(_layernorm(h)).astype(_BF16)

    proj_ln(0, 0)
    attn_steps(2, None, ((GB - 1) * UB, NQ - 1))

    def p3_step(i, slot, do_proj):
        hid = jnp.dot(y_v[slot], w1_v[...], preferred_element_type=_F32)
        hid = jax.nn.gelu(hid + b1_v[...].astype(_F32).reshape(1, F), approximate=True).astype(_BF16)
        if do_proj:
            proj_ln(i + 1, 1 - slot)
        r = jnp.dot(hid, w2_v[...], preferred_element_type=_F32)
        o_v[slot] = (h_v[slot] + (r + b2_v[...].astype(_F32).reshape(1, D))).astype(_BF16)
        out_copy(i, slot).start()

    def p3_body(i, carry):
        slot = i % 2

        @pl.when(i >= 2)
        def _():
            out_copy(i - 2, slot).wait()

        p3_step(i, slot, True)
        return carry

    lax.fori_loop(0, NT - 1, p3_body, 0)
    out_copy(NT - 3, (NT - 1) % 2).wait()
    p3_step(NT - 1, (NT - 1) % 2, False)
    out_copy(NT - 2, 0).wait()
    out_copy(NT - 1, 1).wait()


@jax.jit
def pallas_sequential_preLN__softmax_full_mha__mixer_channel_mlp__prompt_kernel(
    A_x: jax.Array,
    A_wqkv: jax.Array,
    A_wo: jax.Array,
    B_x: jax.Array,
    B_w1: jax.Array,
    B_b1: jax.Array,
    B_w2: jax.Array,
    B_b2: jax.Array,
):
    del B_x
    assert A_x.shape == (1, S, D)
    any_spec = pl.BlockSpec(memory_space=pl.ANY)
    out = pl.pallas_call(
        _kernel,
        out_shape=jax.ShapeDtypeStruct((S, D), A_x.dtype),
        in_specs=[any_spec] * 7,
        out_specs=any_spec,
        scratch_shapes=[
            pltpu.VMEM((S, D), _BF16),
            pltpu.VMEM((D, 3 * D), _BF16),
            pltpu.VMEM((D, D), _BF16),
            pltpu.VMEM((D, F), _BF16),
            pltpu.VMEM((F, D), _BF16),
            pltpu.VMEM((2, TQ, D), _BF16),
            pltpu.VMEM((G, S, 128), _BF16),
            pltpu.VMEM((NQ, D, TQ), _BF16),
            pltpu.VMEM((NQ, D, TQ), _BF16),
            pltpu.VMEM((NT, D, TM), _BF16),
            pltpu.VMEM((S, TQ), _F32),
            pltpu.VMEM((S, TQ), _F32),
            pltpu.VMEM((S, TQ), _F32),
            pltpu.VMEM((S, TQ), _F32),
            pltpu.VMEM((8, TQ), _F32),
            pltpu.VMEM((2, TM, D), _F32),
            pltpu.VMEM((2, TM, D), _BF16),
            pltpu.VMEM((2, TM, D), _BF16),
            pltpu.VMEM((F,), _BF16),
            pltpu.VMEM((D,), _BF16),
            pltpu.SemaphoreType.DMA((NQ + NWCH + 5,)),
            pltpu.SemaphoreType.DMA((2,)),
        ],
        compiler_params=pltpu.CompilerParams(vmem_limit_bytes=110 * 1024 * 1024, disable_bounds_checks=True, disable_semaphore_checks=True),
    )(A_x.reshape(S, D), A_wqkv, A_wo, B_w1, B_b1, B_w2, B_b2)
    return out.reshape(1, S, D)
```

```python
import math

import jax
import jax.numpy as jnp
from jax import lax
import jax.experimental.pallas as pl
import jax.experimental.pallas.tpu as pltpu

S = 2048
D = 1024
H = 32
DH = D // H
F = 3584
G = H // 4
TQ = 256
NQ = S // TQ
CK = 128
NC = S // CK
WCHUNKS = ((0, 256), (256, 256), (512, 512), (2048, 512), (2560, 512), (1024, 512), (1536, 512))
X1POS = 6
NWCH = len(WCHUNKS)
LAG = 1
GL = 4
TM = 128
NT = S // TM
GPB = 4
GB = G // GPB
NU = GB * NQ
UB = 4 * GPB
EPS = 1e-5
QSCALE = (DH ** -0.5) * math.log2(math.e)

_F32 = jnp.float32
_BF16 = jnp.bfloat16


def _layernorm(x):
    m = jnp.mean(x, axis=-1, keepdims=True)
    xc = x - m
    v = jnp.mean(xc * xc, axis=-1, keepdims=True)
    return xc * lax.rsqrt(v + EPS)


def _kernel(x_hbm, wqkv_hbm, wo_hbm, w1_hbm, b1_hbm, w2_hbm, b2_hbm, out_hbm,
            x_v, wqkv_v, wo_v, w1_v, w2_v,
            xn_v, k_v, qt_v, vt_v, ot_v,
            s0, s1, s2, s3, m_v,
            h_v, y_v, o_v, b1_v, b2_v,
            in_sem, o_sem):
    sbuf = (s0, s1, s2, s3)

    def x_copy(i):
        return pltpu.make_async_copy(
            x_hbm.at[pl.ds(i * TQ, TQ), :], x_v.at[pl.ds(i * TQ, TQ), :], in_sem.at[i])

    def wq_copy(c):
        c0, n = WCHUNKS[c]
        return pltpu.make_async_copy(
            wqkv_hbm.at[:, pl.ds(c0, n)], wqkv_v.at[:, pl.ds(c0, n)], in_sem.at[NQ + c])

    def w_copies():
        pairs = ((wo_hbm, wo_v), (w1_hbm, w1_v), (w2_hbm, w2_v), (b1_hbm, b1_v.at[pl.ds(0, F)]), (b2_hbm, b2_v.at[pl.ds(0, D)]))
        return [pltpu.make_async_copy(src, dst, in_sem.at[NQ + NWCH + k])
                for k, (src, dst) in enumerate(pairs)]

    def out_copy(i, slot):
        return pltpu.make_async_copy(
            o_v.at[slot], out_hbm.at[pl.ds(i * TM, TM), :], o_sem.at[slot])

    x_copy(0).start()
    for c in range(NWCH):
        if c == X1POS:
            x_copy(1).start()
        wq_copy(c).start()
    for i in range(2, NQ):
        x_copy(i).start()
    for cp in w_copies():
        cp.start()

    s2[...] = jnp.zeros_like(s2)
    s3[...] = jnp.zeros_like(s3)
    m_v[...] = jnp.zeros_like(m_v)

    def ln_x(i):
        row = pl.multiple_of(i * TQ, TQ)
        return _layernorm(x_v[pl.ds(row, TQ), :].astype(_F32)).astype(_BF16)

    def store_qkv_cols(i, r, col0):
        n = r.shape[1]
        row = pl.multiple_of(i * TQ, TQ)
        for sec in range(3):
            lo, hi = max(col0, sec * D), min(col0 + n, (sec + 1) * D)
            if lo >= hi:
                continue
            part = r[:, lo - col0:hi - col0]
            a, b = lo - sec * D, hi - sec * D
            if sec == 0:
                qt_v[i, a:b, :] = (part * QSCALE).T.astype(_BF16)
            elif sec == 1:
                for g in range(a // 128, b // 128):
                    k_v[g, pl.ds(row, TQ), :] = part[:, g * 128 - a:(g + 1) * 128 - a].astype(_BF16)
            else:
                vt_v[i, a:b, :] = part.T.astype(_BF16)

    x_copy(0).wait()
    xn0 = ln_x(0)
    pending = None
    for c in range(NWCH):
        wq_copy(c).wait()
        if c == NWCH - 1:
            x_copy(1).wait()
        c0, n = WCHUNKS[c]
        r = jnp.dot(xn0, wqkv_v[:, c0:c0 + n], preferred_element_type=_F32)
        if pending is not None:
            store_qkv_cols(0, *pending)
            pending = None
        if c < NWCH - 1 and not (D <= c0 < 2 * D):
            pending = (r, c0)
        else:
            store_qkv_cols(0, r, c0)
    xn_v[1] = ln_x(1)

    def p1_body(i, carry):
        @pl.when(i + 1 < NQ)
        def _():
            x_copy(i + 1).wait()
        xn = xn_v[i % 2]
        for sec in (0, 2, 1):
            r = jnp.dot(xn, wqkv_v[:, sec * D:(sec + 1) * D], preferred_element_type=_F32)
            store_qkv_cols(i, r, sec * D)
        xn_v[(i + 1) % 2] = ln_x(jnp.minimum(i + 1, NQ - 1))
        return carry

    lax.fori_loop(1, NQ, p1_body, 0)

    zeros32 = jnp.zeros((DH, TQ), _BF16)

    def q_weights(h, j, qi):
        row = pl.multiple_of(h * DH, DH)
        qt = qt_v[qi, pl.ds(row, DH), :]
        return jnp.concatenate([qt if jj == j else zeros32 for jj in range(4)], axis=0)

    def qk_chunk(g, w, c, slot, mx):
        s = jnp.dot(k_v[g, c * CK:(c + 1) * CK, :], w, preferred_element_type=_F32)
        sbuf[slot][c * CK:(c + 1) * CK, :] = s
        cm = jnp.max(s.reshape(CK // 8, 8, TQ), axis=0)
        return cm if mx is None else jnp.maximum(mx, cm)

    def sm_chunk(c, slot, m, l):
        p = jnp.exp2(sbuf[slot][c * CK:(c + 1) * CK, :] - m)
        cl = jnp.sum(p.reshape(CK // 8, 8, TQ), axis=0)
        return (cl if l is None else l + cl), p.astype(_BF16)

    def pv_chunk(h, c, pb, o):
        row = pl.multiple_of(h * DH, DH)
        t, off = divmod(c * CK, TQ)
        vt = vt_v[t, pl.ds(row, DH), off:off + CK]
        co = jnp.dot(vt, pb, preferred_element_type=_F32)
        return co if o is None else o + co

    def attn_steps(n_units, cur, prev):
        ms = [m_v[0:1, :], m_v[1:2, :]]
        mx, ls, os_, ps, ws, hist_l, hist_m = {}, {}, {}, {}, {}, {}, {}

        def sm_unit(n):
            return (prev[0] + UB - 2 + n, prev[1]) if n < 2 else (cur[0] + n - 2, cur[1])

        T = n_units * NC
        for t in range(T + LAG):
            if t < T:
                n, c = divmod(t, NC)
                if cur is not None:
                    if c == 0:
                        ws[n] = q_weights(cur[0] + n, n % 4, cur[1])
                    mx[n] = qk_chunk(cur[0] // 4 + n // 4, ws[n], c, n % 4, mx.get(n))
                    hist_m[t] = mx[n]
                    if c == NC - 1:
                        ms.append(jnp.max(mx[n], axis=0, keepdims=True))
                m = ms[n]
                if t >= GL:
                    m = m + hist_l[t - GL][0:1, :] * 0.0
                    if cur is not None:
                        m = m + hist_m[t - GL][0:1, :] * 0.0
                ls[n], ps[t] = sm_chunk(c, (n + 2) % 4, m, ls.get(n))
                hist_l[t] = ls[n]
            if t >= LAG:
                n, c = divmod(t - LAG, NC)
                h, qi = sm_unit(n)
                os_[n] = pv_chunk(h, c, ps.pop(t - LAG), os_.get(n))
                if c == NC - 1:
                    l = jnp.sum(ls[n], axis=0, keepdims=True)
                    row = pl.multiple_of(h * DH, DH)
                    on = (os_[n] * (1.0 / l)).astype(_BF16)
                    for hf in range(TQ // TM):
                        ot_v[qi * (TQ // TM) + hf, pl.ds(row, DH), :] = on[:, hf * TM:(hf + 1) * TM]
        if cur is not None:
            m_v[0:1, :] = ms[n_units]
            m_v[1:2, :] = ms[n_units + 1]

    def p2_body(u, carry):
        up = jnp.maximum(u - 1, 0)
        attn_steps(UB, ((u % GB) * UB, u // GB), ((up % GB) * UB, up // GB))
        return carry

    lax.fori_loop(0, NU, p2_body, 0)

    for cp in w_copies():
        cp.wait()

    def proj_ln(i, slot):
        row = pl.multiple_of(i * TM, TM)
        o = ot_v[i].T
        a = jnp.dot(o, wo_v[...], preferred_element_type=_F32)
        h = x_v[pl.ds(row, TM), :].astype(_F32) + a
        h_v[slot] = h
        y_v[slot] = _layernorm(_layernorm(h)).astype(_BF16)

    proj_ln(0, 0)
    attn_steps(2, None, ((GB - 1) * UB, NQ - 1))

    def p3_step(i, slot, do_proj):
        hid = jnp.dot(y_v[slot], w1_v[...], preferred_element_type=_F32)
        hid = jax.nn.gelu(hid + b1_v[0:F].astype(_F32).reshape(1, F), approximate=True).astype(_BF16)
        if do_proj:
            proj_ln(i + 1, 1 - slot)
        r = jnp.dot(hid, w2_v[...], preferred_element_type=_F32)
        o_v[slot] = (h_v[slot] + (r + b2_v[0:D].astype(_F32).reshape(1, D))).astype(_BF16)
        out_copy(i, slot).start()

    def p3_body(i, carry):
        slot = i % 2

        @pl.when(i >= 2)
        def _():
            out_copy(i - 2, slot).wait()

        p3_step(i, slot, True)
        return carry

    lax.fori_loop(0, NT - 1, p3_body, 0)
    out_copy(NT - 3, (NT - 1) % 2).wait()
    p3_step(NT - 1, (NT - 1) % 2, False)
    out_copy(NT - 2, 0).wait()
    out_copy(NT - 1, 1).wait()


@jax.jit
def pallas_sequential_preLN__softmax_full_mha__mixer_channel_mlp__prompt_kernel(
    A_x: jax.Array,
    A_wqkv: jax.Array,
    A_wo: jax.Array,
    B_x: jax.Array,
    B_w1: jax.Array,
    B_b1: jax.Array,
    B_w2: jax.Array,
    B_b2: jax.Array,
):
    del B_x
    assert A_x.shape == (1, S, D)
    any_spec = pl.BlockSpec(memory_space=pl.ANY)
    out = pl.pallas_call(
        _kernel,
        out_shape=jax.ShapeDtypeStruct((S, D), A_x.dtype),
        in_specs=[any_spec] * 7,
        out_specs=any_spec,
        scratch_shapes=[
            pltpu.VMEM((S, D), _BF16),
            pltpu.VMEM((D, 3 * D), _BF16),
            pltpu.VMEM((D, D), _BF16),
            pltpu.VMEM((D, F), _BF16),
            pltpu.VMEM((F, D), _BF16),
            pltpu.VMEM((2, TQ, D), _BF16),
            pltpu.VMEM((G, S, 128), _BF16),
            pltpu.VMEM((NQ, D, TQ), _BF16),
            pltpu.VMEM((NQ, D, TQ), _BF16),
            pltpu.VMEM((NT, D, TM), _BF16),
            pltpu.VMEM((S, TQ), _F32),
            pltpu.VMEM((S, TQ), _F32),
            pltpu.VMEM((S, TQ), _F32),
            pltpu.VMEM((S, TQ), _F32),
            pltpu.VMEM((8, TQ), _F32),
            pltpu.VMEM((2, TM, D), _F32),
            pltpu.VMEM((2, TM, D), _BF16),
            pltpu.VMEM((2, TM, D), _BF16),
            pltpu.VMEM((4096,), _BF16),
            pltpu.VMEM((2048,), _BF16),
            pltpu.SemaphoreType.DMA((NQ + NWCH + 5,)),
            pltpu.SemaphoreType.DMA((2,)),
        ],
        compiler_params=pltpu.CompilerParams(vmem_limit_bytes=110 * 1024 * 1024, disable_bounds_checks=True, disable_semaphore_checks=True),
    )(A_x.reshape(S, D), A_wqkv, A_wo, B_w1, B_b1, B_w2, B_b2)
    return out.reshape(1, S, D)
```

```python
import math

import jax
import jax.numpy as jnp
from jax import lax
import jax.experimental.pallas as pl
import jax.experimental.pallas.tpu as pltpu

S = 2048
D = 1024
H = 32
DH = D // H
F = 3584
G = H // 4
TQ = 256
NQ = S // TQ
CK = 128
NC = S // CK
WCHUNKS = ((0, 256), (256, 256), (512, 512), (2048, 512), (2560, 512), (1024, 512), (1536, 512))
X1POS = 6
NWCH = len(WCHUNKS)
LAG = 1
GL = 4
TM = 128
NT = S // TM
GPB = 4
GB = G // GPB
NU = GB * NQ
UB = 4 * GPB
EPS = 1e-5
QSCALE = (DH ** -0.5) * math.log2(math.e)

_F32 = jnp.float32
_BF16 = jnp.bfloat16


def _layernorm(x):
    m = jnp.mean(x, axis=-1, keepdims=True)
    xc = x - m
    v = jnp.mean(xc * xc, axis=-1, keepdims=True)
    return xc * lax.rsqrt(v + EPS)


def _kernel(x_hbm, wqkv_hbm, wo_hbm, w1_hbm, b1_hbm, w2_hbm, b2_hbm, out_hbm,
            x_v, wqkv_v, wo_v, w1_v, w2_v,
            xn_v, k_v, qt_v, vt_v, ot_v,
            s0, s1, s2, s3, m_v,
            h_v, y_v, o_v, b1_v, b2_v,
            in_sem, o_sem):
    sbuf = (s0, s1, s2, s3)

    def x_copy(i):
        return pltpu.make_async_copy(
            x_hbm.at[pl.ds(i * TQ, TQ), :], x_v.at[pl.ds(i * TQ, TQ), :], in_sem.at[i])

    def wq_copy(c):
        c0, n = WCHUNKS[c]
        return pltpu.make_async_copy(
            wqkv_hbm.at[:, pl.ds(c0, n)], wqkv_v.at[:, pl.ds(c0, n)], in_sem.at[NQ + c])

    def w_copies():
        pairs = ((wo_hbm, wo_v), (w1_hbm, w1_v), (w2_hbm, w2_v),
                 (b1_hbm, b1_v.at[pl.ds(0, F)]), (b2_hbm, b2_v.at[pl.ds(0, D)]))
        return [pltpu.make_async_copy(src, dst, in_sem.at[NQ + NWCH + k])
                for k, (src, dst) in enumerate(pairs)]

    def out_copy(i, slot):
        return pltpu.make_async_copy(
            o_v.at[slot], out_hbm.at[pl.ds(i * TM, TM), :], o_sem.at[slot])

    x_copy(0).start()
    for c in range(NWCH):
        if c == X1POS:
            x_copy(1).start()
        wq_copy(c).start()
    for i in range(2, NQ):
        x_copy(i).start()
    for cp in w_copies():
        cp.start()

    s2[...] = jnp.zeros_like(s2)
    s3[...] = jnp.zeros_like(s3)
    m_v[...] = jnp.zeros_like(m_v)

    def ln_x(i):
        row = pl.multiple_of(i * TQ, TQ)
        return _layernorm(x_v[pl.ds(row, TQ), :].astype(_F32)).astype(_BF16)

    def store_qkv_cols(i, r, col0):
        n = r.shape[1]
        row = pl.multiple_of(i * TQ, TQ)
        for sec in range(3):
            lo, hi = max(col0, sec * D), min(col0 + n, (sec + 1) * D)
            if lo >= hi:
                continue
            part = r[:, lo - col0:hi - col0]
            a, b = lo - sec * D, hi - sec * D
            if sec == 0:
                qt_v[i, a:b, :] = (part * QSCALE).T.astype(_BF16)
            elif sec == 1:
                for g in range(a // 128, b // 128):
                    k_v[g, pl.ds(row, TQ), :] = part[:, g * 128 - a:(g + 1) * 128 - a].astype(_BF16)
            else:
                vt_v[i, a:b, :] = part.T.astype(_BF16)

    x_copy(0).wait()
    xn0 = ln_x(0)
    pending = None
    for c in range(NWCH):
        wq_copy(c).wait()
        if c == NWCH - 1:
            x_copy(1).wait()
        c0, n = WCHUNKS[c]
        r = jnp.dot(xn0, wqkv_v[:, c0:c0 + n], preferred_element_type=_F32)
        if pending is not None:
            store_qkv_cols(0, *pending)
            pending = None
        if c < NWCH - 1 and not (D <= c0 < 2 * D):
            pending = (r, c0)
        else:
            store_qkv_cols(0, r, c0)
    xn_v[1] = ln_x(1)

    def p1_body(i, carry):
        @pl.when(i + 1 < NQ)
        def _():
            x_copy(i + 1).wait()
        xn = xn_v[i % 2]
        for sec in (0, 2, 1):
            r = jnp.dot(xn, wqkv_v[:, sec * D:(sec + 1) * D], preferred_element_type=_F32)
            store_qkv_cols(i, r, sec * D)
        xn_v[(i + 1) % 2] = ln_x(jnp.minimum(i + 1, NQ - 1))
        return carry

    lax.fori_loop(1, NQ, p1_body, 0)

    zeros32 = jnp.zeros((DH, TQ), _BF16)

    def q_weights(h, j, qi):
        row = pl.multiple_of(h * DH, DH)
        qt = qt_v[qi, pl.ds(row, DH), :]
        return jnp.concatenate([qt if jj == j else zeros32 for jj in range(4)], axis=0)

    def qk_chunk(g, w, c, slot, mx):
        s = jnp.dot(k_v[g, c * CK:(c + 1) * CK, :], w, preferred_element_type=_F32)
        sbuf[slot][c * CK:(c + 1) * CK, :] = s
        cm = jnp.max(s.reshape(CK // 8, 8, TQ), axis=0)
        return cm if mx is None else jnp.maximum(mx, cm)

    def sm_chunk(c, slot, m, l):
        p = jnp.exp2(sbuf[slot][c * CK:(c + 1) * CK, :] - m)
        cl = jnp.sum(p.reshape(CK // 8, 8, TQ), axis=0)
        return (cl if l is None else l + cl), p.astype(_BF16)

    def pv_chunk(h, c, pb, o):
        row = pl.multiple_of(h * DH, DH)
        t, off = divmod(c * CK, TQ)
        vt = vt_v[t, pl.ds(row, DH), off:off + CK]
        co = jnp.dot(vt, pb, preferred_element_type=_F32)
        return co if o is None else o + co

    def attn_steps(n_units, cur, prev):
        ms = [m_v[0:1, :], m_v[1:2, :]]
        mx, ls, os_, ps, ws, hist_l, hist_m = {}, {}, {}, {}, {}, {}, {}

        def sm_unit(n):
            return (prev[0] + UB - 2 + n, prev[1]) if n < 2 else (cur[0] + n - 2, cur[1])

        T = n_units * NC
        for t in range(T + LAG):
            if t < T:
                n, c = divmod(t, NC)
                if cur is not None:
                    if c == 0:
                        ws[n] = q_weights(cur[0] + n, n % 4, cur[1])
                    mx[n] = qk_chunk(cur[0] // 4 + n // 4, ws[n], c, n % 4, mx.get(n))
                    hist_m[t] = mx[n]
                    if c == NC - 1:
                        ms.append(jnp.max(mx[n], axis=0, keepdims=True))
                m = ms[n]
                if t >= GL:
                    m = m + hist_l[t - GL][0:1, :] * 0.0
                    if cur is not None:
                        m = m + hist_m[t - GL][0:1, :] * 0.0
                ls[n], ps[t] = sm_chunk(c, (n + 2) % 4, m, ls.get(n))
                hist_l[t] = ls[n]
            if t >= LAG:
                n, c = divmod(t - LAG, NC)
                h, qi = sm_unit(n)
                os_[n] = pv_chunk(h, c, ps.pop(t - LAG), os_.get(n))
                if c == NC - 1:
                    l = jnp.sum(ls[n], axis=0, keepdims=True)
                    row = pl.multiple_of(h * DH, DH)
                    on = (os_[n] * (1.0 / l)).astype(_BF16)
                    for hf in range(TQ // TM):
                        ot_v[qi * (TQ // TM) + hf, pl.ds(row, DH), :] = on[:, hf * TM:(hf + 1) * TM]
        if cur is not None:
            m_v[0:1, :] = ms[n_units]
            m_v[1:2, :] = ms[n_units + 1]

    def p2_body(u, carry):
        up = jnp.maximum(u - 1, 0)
        attn_steps(UB, ((u % GB) * UB, u // GB), ((up % GB) * UB, up // GB))
        return carry

    lax.fori_loop(0, NU, p2_body, 0)

    for cp in w_copies():
        cp.wait()

    def proj_ln(i, slot):
        row = pl.multiple_of(i * TM, TM)
        o = ot_v[i].T
        a = jnp.dot(o, wo_v[...], preferred_element_type=_F32)
        h = x_v[pl.ds(row, TM), :].astype(_F32) + a
        h_v[slot] = h
        y_v[slot] = _layernorm(_layernorm(h)).astype(_BF16)

    proj_ln(0, 0)
    attn_steps(2, None, ((GB - 1) * UB, NQ - 1))

    def p3_step(i, slot, do_proj):
        hid = jnp.dot(y_v[slot], w1_v[...], preferred_element_type=_F32)
        hid = jax.nn.gelu(hid + b1_v[0:F].astype(_F32).reshape(1, F), approximate=True).astype(_BF16)
        if do_proj:
            proj_ln(i + 1, 1 - slot)
        r = jnp.dot(hid, w2_v[...], preferred_element_type=_F32)
        o_v[slot] = (h_v[slot] + (r + b2_v[0:D].astype(_F32).reshape(1, D))).astype(_BF16)
        out_copy(i, slot).start()

    def p3_body(i, carry):
        slot = i % 2

        @pl.when(i >= 2)
        def _():
            out_copy(i - 2, slot).wait()

        p3_step(i, slot, True)
        return carry

    lax.fori_loop(0, NT - 1, p3_body, 0)
    out_copy(NT - 3, (NT - 1) % 2).wait()
    p3_step(NT - 1, (NT - 1) % 2, False)
    out_copy(NT - 2, 0).wait()
    out_copy(NT - 1, 1).wait()


@jax.jit
def pallas_sequential_preLN__softmax_full_mha__mixer_channel_mlp__prompt_kernel(
    A_x: jax.Array,
    A_wqkv: jax.Array,
    A_wo: jax.Array,
    B_x: jax.Array,
    B_w1: jax.Array,
    B_b1: jax.Array,
    B_w2: jax.Array,
    B_b2: jax.Array,
):
    del B_x
    assert A_x.shape == (1, S, D)
    any_spec = pl.BlockSpec(memory_space=pl.ANY)
    out = pl.pallas_call(
        _kernel,
        out_shape=jax.ShapeDtypeStruct((S, D), A_x.dtype),
        in_specs=[any_spec] * 7,
        out_specs=any_spec,
        scratch_shapes=[
            pltpu.VMEM((S, D), _BF16),
            pltpu.VMEM((D, 3 * D), _BF16),
            pltpu.VMEM((D, D), _BF16),
            pltpu.VMEM((D, F), _BF16),
            pltpu.VMEM((F, D), _BF16),
            pltpu.VMEM((2, TQ, D), _BF16),
            pltpu.VMEM((G, S, 128), _BF16),
            pltpu.VMEM((NQ, D, TQ), _BF16),
            pltpu.VMEM((NQ, D, TQ), _BF16),
            pltpu.VMEM((NT, D, TM), _BF16),
            pltpu.VMEM((S, TQ), _F32),
            pltpu.VMEM((S, TQ), _F32),
            pltpu.VMEM((S, TQ), _F32),
            pltpu.VMEM((S, TQ), _F32),
            pltpu.VMEM((8, TQ), _F32),
            pltpu.VMEM((2, TM, D), _F32),
            pltpu.VMEM((2, TM, D), _BF16),
            pltpu.VMEM((2, TM, D), _BF16),
            pltpu.VMEM((4096,), _BF16),
            pltpu.VMEM((2048,), _BF16),
            pltpu.SemaphoreType.DMA((NQ + NWCH + 5,)),
            pltpu.SemaphoreType.DMA((2,)),
        ],
        compiler_params=pltpu.CompilerParams(
            vmem_limit_bytes=110 * 1024 * 1024,
            disable_bounds_checks=True,
            disable_semaphore_checks=True,
        ),
    )(A_x.reshape(S, D), A_wqkv, A_wo, B_w1, B_b1, B_w2, B_b2)
    return out.reshape(1, S, D)
```
